```python
import os as _os
_os.environ.setdefault("JAX_PLATFORMS", "cpu")
import jax
import jax.numpy as jnp

def _softmax(x, axis=-1):
    return jax.nn.softmax(x, axis=axis)
def _gelu(x):
    return jax.nn.gelu(x, approximate=True)
def _silu(x):
    return jax.nn.silu(x)
def _sigmoid(x):
    return jax.nn.sigmoid(x)
def _layernorm(x, axis=-1, eps=1e-5):
    m = jnp.mean(x, axis=axis, keepdims=True)
    v = jnp.var(x, axis=axis, keepdims=True)
    return (x - m) / jnp.sqrt(v + eps)
def _scatter_add(tgt, idx, src, axis=0):
    return tgt.at[idx].add(src)
def _segment_sum(src, seg, n):
    return jax.ops.segment_sum(src, seg, n)
class _Rng:
    def __init__(self, key):
        self._k = key
    def _next(self):
        self._k, sub = jax.random.split(self._k)
        return sub
    def normal(self, shape):
        return jax.random.normal(self._next(), shape, dtype=jnp.bfloat16)
    def randint(self, lo, hi, shape):
        return jax.random.randint(self._next(), shape, lo, hi, dtype=jnp.int32)
    def uniform(self, shape, lo=0.0, hi=1.0):
        return jax.random.uniform(self._next(), shape, jnp.bfloat16, lo, hi)
    def permutation(self, n):
        return jax.random.permutation(self._next(), n)


kernel_name = 'concat_heads__linear_kernel_hedgehog__ssm_conv_s5__prompt'

def setup_inputs():
    _rng = _Rng(jax.random.key(int.from_bytes(__import__("os").urandom(4), "little")))
    _w = (lambda a: (lambda t: t.astype(jnp.bfloat16) if jnp.issubdtype(t.dtype, jnp.floating) else t)(jnp.asarray(a)))
    def _A_setup():
        B, S, D, H = 1, 2048, 640, 32
        Dh = D // H
        return {
            "x": _w((lambda *s: _rng.normal(s) * 0.4)(B, S, D)),
            "wqkv": _w((lambda *s: _rng.normal(s) * 0.4)(D, 3 * D)),
            "w_phi": _w((lambda *s: _rng.normal(s) * 0.4)(H, Dh, Dh) * (Dh ** -0.5)),
            "wo": _w((lambda *s: _rng.normal(s) * 0.05)(D, D)),
        }
    _A_in = _A_setup()

    def _B_setup():
        B, S, D = 1, 2048, 640
        P = D
        Lambda_re = -0.5 * jnp.exp((lambda *s: _rng.normal(s) * 0.8)(P))
        Lambda_im = (lambda *s: _rng.normal(s) * 0.8)(P) * 1.0
        B_re = (lambda *s: _rng.normal(s) * 0.8)(P, D) * (D ** -0.5)
        B_im = (lambda *s: _rng.normal(s) * 0.8)(P, D) * (D ** -0.5)
        C_re = (lambda *s: _rng.normal(s) * 0.8)(D, P) * (P ** -0.5)
        C_im = (lambda *s: _rng.normal(s) * 0.8)(D, P) * (P ** -0.5)
        log_dt = (lambda *s: _rng.normal(s) * 0.8)(P) * 0.3 - 2.0
        Dskip = (lambda *s: _rng.normal(s) * 0.8)(D)
        return {
            "x": _w((lambda *s: _rng.normal(s) * 0.05)(B, S, D)),
            "Lambda_re": _w(Lambda_re),
            "Lambda_im": _w(Lambda_im),
            "B_re": _w(B_re),
            "B_im": _w(B_im),
            "C_re": _w(C_re),
            "C_im": _w(C_im),
            "log_dt": _w(log_dt),
            "Dskip": _w(Dskip),
        }
    _B_in = _B_setup()

    return {
        "A_x": _A_in["x"],
        "A_wqkv": _A_in["wqkv"],
        "A_w_phi": _A_in["w_phi"],
        "A_wo": _A_in["wo"],
        "B_x": _B_in["x"],
        "B_Lambda_re": _B_in["Lambda_re"],
        "B_Lambda_im": _B_in["Lambda_im"],
        "B_B_re": _B_in["B_re"],
        "B_B_im": _B_in["B_im"],
        "B_C_re": _B_in["C_re"],
        "B_C_im": _B_in["C_im"],
        "B_log_dt": _B_in["log_dt"],
        "B_Dskip": _B_in["Dskip"],
    }

def reference(A_x, A_wqkv, A_w_phi, A_wo, B_x, B_Lambda_re, B_Lambda_im, B_B_re, B_B_im, B_C_re, B_C_im, B_log_dt, B_Dskip):
    def _A_ref(x, wqkv, w_phi, wo):
        B, S, D = x.shape
        H = 32; Dh = D // H
        qkv = (lambda x, *d: x.transpose(*d))((x @ wqkv).reshape(B, S, 3, H, Dh), 2, 0, 3, 1, 4)
        q, k, v = qkv[0], qkv[1], qkv[2]
        pq = jnp.einsum("bhsd,hdf->bhsf", q, w_phi)
        pk = jnp.einsum("bhsd,hdf->bhsf", k, w_phi)
        phi_q = jnp.concatenate([_softmax(pq, axis=-1), _softmax(-pq, axis=-1)], axis=-1)
        phi_k = jnp.concatenate([_softmax(pk, axis=-1), _softmax(-pk, axis=-1)], axis=-1)
        kv = jnp.einsum("bhsf,bhsd->bhfd", phi_k, v)
        z  = jnp.einsum("bhsf->bhf", phi_k)
        num = jnp.einsum("bhqf,bhfd->bhqd", phi_q, kv)
        den = jnp.einsum("bhqf,bhf->bhq", phi_q, z)[..., None] + 1e-6
        o = num / den
        return (lambda x, *d: x.transpose(*d))(o, 0, 2, 1, 3).reshape(B, S, D) @ wo

    def _B_ref(x, Lambda_re, Lambda_im, B_re, B_im, C_re, C_im, log_dt, Dskip):
        Bsz, L, H = x.shape
        Lam = Lambda_re + 1j * Lambda_im
        Bmat = B_re + 1j * B_im
        Cmat = C_re + 1j * C_im
        dt = jnp.exp(log_dt)
        Lam_bar = jnp.exp(dt * Lam)
        B_bar = ((Lam_bar - 1.0) / Lam)[:, None] * Bmat
        Bu = jnp.einsum("bld,pd->blp", x + 0j, B_bar)
        h = jnp.zeros_like(Bu[:, 0, :])
        hs = []
        for t in range(L):
            h = Lam_bar[None, :] * h + Bu[:, t, :]
            hs.append(h)
        hseq = jnp.stack(hs, 1)
        y = 2.0 * jnp.einsum("blp,dp->bld", hseq, Cmat).real + x * Dskip[None, None, :]
        return y

    a = _A_ref(A_x, A_wqkv, A_w_phi, A_wo)
    b = _B_ref(B_x, B_Lambda_re, B_Lambda_im, B_B_re, B_B_im, B_C_re, B_C_im, B_log_dt, B_Dskip)
    return jnp.concatenate([a, b], axis=-1)
```

```python
import numpy as np

import jax
import jax.numpy as jnp
from jax import lax
import jax.experimental.pallas as pl
import jax.experimental.pallas.tpu as pltpu

S, D, P = 2048, 640, 640
f32, bf16 = jnp.float32, jnp.bfloat16
NT = (((1,), (1,)), ((), ()))
NN = (((1,), (0,)), ((), ()))
TN = (((0,), (0,)), ((), ()))
LOG2E = 1.4426950408889634
TB = [((128 * t) // 80, (128 * t + 127) // 80) for t in range(10)]
TOFF = np.cumsum([0] + [48 * (b1 - b0 + 1) for b0, b1 in TB]).tolist()

CA = 512
CB = 256
NIT = S // CA


def _dot(a, b, dn):
  return lax.dot_general(a, b, dn, preferred_element_type=f32)


def _cmul(ar, ai, br, bi):
  return ar * br - ai * bi, ar * bi + ai * br


def _softmax2(p, C):
  x = p.reshape(16, 5, 8, C)

  def allred(m, op):
    m = op(m, pltpu.roll(m, 4, 1))
    return op(m, pltpu.roll(m, 2, 1))

  mx = allred(jnp.max(x, axis=1), jnp.maximum)[:, None]
  mn = allred(jnp.min(x, axis=1), jnp.minimum)[:, None]
  ep = jnp.exp2(x - mx)
  en = jnp.exp2(mn - x)
  rp = (1.0 / allred(jnp.sum(ep, axis=1), jnp.add))[:, None]
  rn = (1.0 / allred(jnp.sum(en, axis=1), jnp.add))[:, None]
  phi = jnp.concatenate([ep * rp, en * rn], axis=1)
  return phi.reshape(1280, C).astype(bf16)


def _prep_fold(wt_s, wqkv_s, WT_s):
  prev = [None, None]
  for j in range(5):
    r = lax.broadcasted_iota(jnp.int32, (32, 128), 1) + 128 * j
    hr = (r * 3277) >> 16
    E = jnp.where(lax.broadcasted_iota(jnp.int32, (32, 128), 0) == hr, 1.0, 0.0).astype(bf16)
    dr1 = (r - 20 * hr)[0:1, :]
    T = jnp.zeros((20, 128), f32)
    for d in range(20):
      Y = _dot(wt_s[d], E, NN)
      T = jnp.where(dr1 == d, Y, T)
    T2 = pltpu.bitcast(pltpu.pack_elementwise([T, T], packed_dtype=bf16), bf16).astype(f32)
    h2 = lax.broadcasted_iota(jnp.int32, (40, 128), 0) & 1
    hr1 = hr[0:1, :]
    lhs = jnp.concatenate(
        [jnp.where(2 * (3 * j + bb) + h2 == hr1, T2, 0.0) for bb in range(4)], 0).astype(bf16)
    for n in range(2):
      res = _dot(lhs, wqkv_s[:, 640 * n + 128 * j: 640 * n + 128 * j + 128], NT) * LOG2E
      lo = 640 * n + 120 * j
      if j == 0:
        WT_s[lo: lo + 120, :] = res[0:120].astype(bf16)
      else:
        WT_s[lo: lo + 40, :] = (prev[n] + res[0:40]).astype(bf16)
        WT_s[lo + 40: lo + 120, :] = res[40:120].astype(bf16)
      if j < 4:
        prev[n] = res[120:160]
      else:
        WT_s[lo + 120: lo + 160, :] = res[120:160].astype(bf16)
  WT_s[1280:1920, :] = wqkv_s[:, 1280:1920].T


def _kernel(xa_hbm, wqkv_hbm, wt_hbm, wo_hbm, xb_hbm, lre_hbm, lim_hbm, bre_hbm, bim_hbm,
            cre_hbm, cim_hbm, ldt_hbm, dsk_hbm, o_hbm,
            xa_s, wqkv_s, wt_s, wo_s, WT_s, kv_s, kvm_s, oa_s,
            xb_s, v0_s, v1_s, v2_s, v3_s, b_s, c_s, cp_s, tab_s, carry_s, ob_s,
            sem, osem):
  vec_l = [v0_s, v1_s, v2_s, v3_s]
  mk = pltpu.make_async_copy
  cps = [
      mk(lre_hbm, v0_s, sem.at[0]),
      mk(lim_hbm, v1_s, sem.at[1]),
      mk(ldt_hbm, v2_s, sem.at[2]),
      mk(dsk_hbm, v3_s, sem.at[3]),
      mk(wt_hbm, wt_s, sem.at[4]),
      mk(wqkv_hbm, wqkv_s, sem.at[5]),
      mk(cre_hbm, c_s.at[0], sem.at[6]),
      mk(cim_hbm, c_s.at[1], sem.at[7]),
      mk(bre_hbm, b_s.at[0:640], sem.at[8]),
      mk(bim_hbm, b_s.at[640:1280], sem.at[9]),
      mk(xb_hbm.at[0], xb_s, sem.at[10]),
      mk(xa_hbm.at[0], xa_s, sem.at[11]),
      mk(wo_hbm, wo_s, sem.at[12]),
  ]
  for c in cps:
    c.start()

  for c in cps[:4]:
    c.wait()

  def v(i):
    return jnp.broadcast_to(vec_l[i][...].astype(f32).reshape(1, P), (8, P))

  lre, lim, ldt, dsk = v(0), v(1), v(2), v(3)
  dt = jnp.exp(ldt).astype(bf16).astype(f32)
  a = dt * lre
  b = dt * lim
  mag = jnp.exp(a)
  lr, li = mag * jnp.cos(b), mag * jnp.sin(b)
  den = lre * lre + lim * lim
  cr = ((lr - 1.0) * lre + li * lim) / den
  ci = (li * lre - (lr - 1.0) * lim) / den
  j8 = lax.broadcasted_iota(jnp.int32, (8, P), 0)
  pw = [(lr, li)]
  for k in range(7):
    pw.append(_cmul(*pw[-1], lr, li))
  pr, pi = pw[0]
  for k in range(1, 8):
    pr = jnp.where(j8 == k, pw[k][0], pr)
    pi = jnp.where(j8 == k, pw[k][1], pi)
  tab_s[0] = pr
  tab_s[1] = pi
  for n, s in enumerate((1, 2, 4)):
    tab_s[2 + 2 * n] = jnp.where(j8 >= s, pw[s - 1][0], 0.0)
    tab_s[3 + 2 * n] = jnp.where(j8 >= s, pw[s - 1][1], 0.0)
  tab_s[8] = dsk
  carry_s[...] = jnp.zeros_like(carry_s)
  kv_s[...] = jnp.zeros_like(kv_s)

  cps[4].wait()
  cps[5].wait()
  _prep_fold(wt_s, wqkv_s, WT_s)

  cps[6].wait()
  cps[7].wait()
  cre = c_s[0].astype(f32)
  cim = c_s[1].astype(f32)
  cr1 = cr[0:1] * 2.0
  ci1 = ci[0:1] * 2.0
  cp_s[:, 0:640] = (cre * cr1 - cim * ci1).astype(bf16)
  cp_s[:, 640:1280] = (-(cre * ci1 + cim * cr1)).astype(bf16)
  for c in cps[8:12]:
    c.wait()

  def out_b(i):
    r0 = pl.multiple_of(i * CB, CB)
    return mk(ob_s.at[pl.ds(r0, CB)], o_hbm.at[0, pl.ds(r0, CB), 640:1280], osem.at[0])

  def out_a(i):
    r0 = pl.multiple_of(i * CA, CA)
    return mk(oa_s.at[pl.ds(r0, CA)], o_hbm.at[0, pl.ds(r0, CA), 0:640], osem.at[1])

  def bchunk(i):
    r0 = pl.multiple_of(i * CB, CB)
    x = xb_s[pl.ds(r0, CB), :]
    u = _dot(x, b_s[...], NT)
    G = CB // 8
    hr_l, hi_l = [], []
    for c in range(5):
      sl = slice(128 * c, 128 * c + 128)
      vr = u[:, sl].reshape(G, 8, 128)
      vi = u[:, 640 + 128 * c: 640 + 128 * c + 128].reshape(G, 8, 128)
      for n, s in enumerate((1, 2, 4)):
        mr = tab_s[2 + 2 * n][:, sl][None]
        mi = tab_s[3 + 2 * n][:, sl][None]
        rr = pltpu.roll(vr, s, 1)
        ri = pltpu.roll(vi, s, 1)
        vr, vi = vr + (mr * rr - mi * ri), vi + (mr * ri + mi * rr)
      pr_ = tab_s[0][:, sl]
      pi_ = tab_s[1][:, sl]
      cr_ = carry_s[0][:, sl]
      ci_ = carry_s[1][:, sl]
      outr, outi = [], []
      for g in range(G):
        hr = vr[g] + (pr_ * cr_ - pi_ * ci_)
        hi = vi[g] + (pr_ * ci_ + pi_ * cr_)
        outr.append(hr)
        outi.append(hi)
        cr_ = jnp.broadcast_to(hr[7:8, :], (8, 128))
        ci_ = jnp.broadcast_to(hi[7:8, :], (8, 128))
      carry_s[0, :, sl] = cr_
      carry_s[1, :, sl] = ci_
      hr_l.append(jnp.concatenate(outr, 0))
      hi_l.append(jnp.concatenate(outi, 0))
    h = jnp.concatenate(hr_l + hi_l, 1).astype(bf16)
    y = _dot(h, cp_s[...], NT)
    y = y + x.astype(f32) * tab_s[8][0:1, :]
    ob_s[pl.ds(r0, CB), :] = y
    out_b(i).start()

  def kchunk(i):
    r0 = pl.multiple_of(i * CA, CA)
    x = xa_s[pl.ds(r0, CA), :]
    pkv = _dot(WT_s[640:1920, :], x, NT)
    phi = _softmax2(pkv[0:640], CA)
    vv = pkv[640:1280].reshape(16, 40, CA)
    vext = jnp.concatenate([vv, jnp.ones((16, 8, CA), f32)], axis=1).reshape(768, CA).astype(bf16)
    for t, (b0, b1) in enumerate(TB):
      r = _dot(vext[48 * b0: 48 * (b1 + 1)], phi[128 * t: 128 * t + 128], NT)
      kv_s[TOFF[t]: TOFF[t + 1], :] += r

  def qchunk(i):
    r0 = pl.multiple_of(i * CA, CA)
    x = xa_s[pl.ds(r0, CA), :]
    pq = _dot(WT_s[0:640, :], x, NT)
    phi = _softmax2(pq, CA)
    acc = [None] * 16
    for t, (b0, b1) in enumerate(TB):
      r = _dot(kvm_s[TOFF[t]: TOFF[t + 1], :], phi[128 * t: 128 * t + 128], NN)
      for bb in range(b1 - b0 + 1):
        piece = r[48 * bb: 48 * bb + 48]
        acc[b0 + bb] = piece if acc[b0 + bb] is None else acc[b0 + bb] + piece
    sub = lax.broadcasted_iota(jnp.int32, (8, CA), 0)
    outs = []
    for b in range(16):
      rd = 1.0 / (acc[b][40:48] + 1e-6)
      rs = pltpu.roll(rd, 4, 0)
      r0_ = jnp.where(sub < 4, rd, rs)
      r1_ = jnp.where(sub < 4, rs, rd)
      sc = jnp.concatenate([r0_, r0_, rd, r1_, r1_], 0)
      outs.append(acc[b][0:40] * sc)
    oT = jnp.concatenate(outs, 0).astype(bf16)
    oa_s[pl.ds(r0, CA), :] = _dot(oT, wo_s[...], TN)
    out_a(i).start()

  def body1(i, _):
    kchunk(i)
    bchunk(i)
    return _

  lax.fori_loop(0, NIT, body1, 0)

  for t, (b0, b1) in enumerate(TB):
    kap = lax.broadcasted_iota(jnp.int32, (48, 128), 1) + 128 * t
    kb = (kap * 13108) >> 20
    hcol = 2 * kb + (kap & 1)
    rr = lax.broadcasted_iota(jnp.int32, (48, 128), 0)
    hin = jnp.where(rr < 40, jnp.where(rr < 20, 0, 1), jnp.where(rr < 44, 0, 1))
    for bb in range(b1 - b0 + 1):
      o = TOFF[t] + 48 * bb
      kvm_s[o: o + 48, :] = jnp.where(hcol == 2 * (b0 + bb) + hin, kv_s[o: o + 48, :], 0.0).astype(bf16)
  cps[12].wait()

  def body2(i, _):
    qchunk(i)
    bchunk(NIT + i)
    return _

  lax.fori_loop(0, NIT, body2, 0)

  for i in range(2 * NIT):
    out_b(i).wait()
  for i in range(NIT):
    out_a(i).wait()


@jax.jit
def pallas_concat_heads__linear_kernel_hedgehog__ssm_conv_s5__prompt_kernel(
    A_x: jax.Array,
    A_wqkv: jax.Array,
    A_w_phi: jax.Array,
    A_wo: jax.Array,
    B_x: jax.Array,
    B_Lambda_re: jax.Array,
    B_Lambda_im: jax.Array,
    B_B_re: jax.Array,
    B_B_im: jax.Array,
    B_C_re: jax.Array,
    B_C_im: jax.Array,
    B_log_dt: jax.Array,
    B_Dskip: jax.Array,
):
  wt = jnp.transpose(A_w_phi, (1, 2, 0))
  return pl.pallas_call(
      _kernel,
      out_shape=jax.ShapeDtypeStruct((1, S, 2 * D), f32),
      in_specs=[pl.BlockSpec(memory_space=pl.ANY)] * 13,
      out_specs=pl.BlockSpec(memory_space=pl.ANY),
      scratch_shapes=[
          pltpu.VMEM((S, D), bf16), pltpu.VMEM((D, 1920), bf16), pltpu.VMEM((20, 20, 32), bf16),
          pltpu.VMEM((D, D), bf16), pltpu.VMEM((1920, D), bf16), pltpu.VMEM((TOFF[-1], 128), f32),
          pltpu.VMEM((TOFF[-1], 128), bf16), pltpu.VMEM((S, D), f32),
          pltpu.VMEM((S, D), bf16), pltpu.VMEM((P,), bf16), pltpu.VMEM((P,), bf16),
          pltpu.VMEM((P,), bf16), pltpu.VMEM((P,), bf16), pltpu.VMEM((1280, D), bf16),
          pltpu.VMEM((2, D, P), bf16), pltpu.VMEM((D, 1280), bf16), pltpu.VMEM((9, 8, P), f32),
          pltpu.VMEM((2, 8, P), f32), pltpu.VMEM((S, D), f32),
          pltpu.SemaphoreType.DMA((13,)), pltpu.SemaphoreType.DMA((2,)),
      ],
      compiler_params=pltpu.CompilerParams(vmem_limit_bytes=100 * 2**20),
  )(A_x, A_wqkv, wt, A_wo, B_x, B_Lambda_re, B_Lambda_im, B_B_re, B_B_im, B_C_re, B_C_im,
    B_log_dt, B_Dskip)
```

```python
import numpy as np

import jax
import jax.numpy as jnp
from jax import lax
import jax.experimental.pallas as pl
import jax.experimental.pallas.tpu as pltpu

S, D, P = 2048, 640, 640
f32, bf16 = jnp.float32, jnp.bfloat16
NT = (((1,), (1,)), ((), ()))
NN = (((1,), (0,)), ((), ()))
LOG2E = 1.4426950408889634
TB = [((128 * t) // 80, (128 * t + 127) // 80) for t in range(10)]
TOFF = np.cumsum([0] + [48 * (b1 - b0 + 1) for b0, b1 in TB]).tolist()

CA = 512
CB = CA // 2
NIT = S // CA
BG = ((0, 1), (1, 3), (3, 5))
ORDER1 = "B012,Y0,PK,V0,Y1,PQ,V1,Y2,B34,Y3,KV,Y4".split(",")
ORDER2 = "NUM,Y0,Y1,W0,Y2,W1,Y3,W2,Y4,W3,W4".split(",")
INJ1 = (0, 0, 0, 0, 0)
INJ2 = (1, 2, 1, 1, 1)


def _dot(a, b, dn):
  return lax.dot_general(a, b, dn, preferred_element_type=f32)


def _mo(x, n):
  return x if isinstance(x, int) else pl.multiple_of(x, n)


def _cmul(ar, ai, br, bi):
  return ar * br - ai * bi, ar * bi + ai * br


def _iota(shape, dim):
  return lax.broadcasted_iota(jnp.int32, shape, dim)


def _softmax2(p):
  c = p.shape[1]
  x = p.reshape(16, 5, 8, c)

  def allred(m, op):
    m = op(m, pltpu.roll(m, 4, 1))
    return op(m, pltpu.roll(m, 2, 1))[:, None]

  mx = allred(jnp.max(x, axis=1), jnp.maximum)
  mn = allred(jnp.min(x, axis=1), jnp.minimum)
  ep = jnp.exp2(x - mx)
  en = jnp.exp2(mn - x)
  rp = 1.0 / allred(jnp.sum(ep, axis=1), jnp.add)
  rn = 1.0 / allred(jnp.sum(en, axis=1), jnp.add)
  phi = jnp.concatenate([ep * rp, en * rn], axis=1)
  return phi.reshape(1280, c).astype(bf16)


def _fold_lhs(wt_s, j):
  r = _iota((32, 128), 1) + 128 * j
  hr = (r * 3277) >> 16
  e = jnp.where(_iota((32, 128), 0) == hr, 1.0, 0.0).astype(bf16)
  dr1 = (r - 20 * hr)[0:1, :]
  t = jnp.zeros((20, 128), f32)
  for d in range(20):
    t = jnp.where(dr1 == d, _dot(wt_s[d], e, NN), t)
  dup = jnp.where(_iota((40, 20), 0) >> 1 == _iota((40, 20), 1), 1.0, 0.0).astype(bf16)
  t2 = _dot(dup, t.astype(bf16), NN)
  h2 = _iota((40, 128), 0) & 1
  hr1 = hr[0:1, :]
  return jnp.concatenate(
      [jnp.where(2 * (3 * j + bb) + h2 == hr1, t2, 0.0) for bb in range(4)], 0).astype(bf16)


def _fold(lhs_s, w_ref, wt_out, n):
  prev = None
  for j in range(5):
    res = _dot(lhs_s[j], w_ref[:, 128 * j: 128 * j + 128], NT) * LOG2E
    lo = 640 * n + 120 * j
    if j == 0:
      wt_out[lo: lo + 120, :] = res[0:120].astype(bf16)
    else:
      wt_out[lo: lo + 40, :] = (prev + res[0:40]).astype(bf16)
      wt_out[lo + 40: lo + 120, :] = res[40:120].astype(bf16)
    if j < 4:
      prev = res[120:160]
    else:
      wt_out[lo + 120: lo + 160, :] = res[120:160].astype(bf16)


def _kernel(xa_hbm, wqkv_hbm, wt_hbm, wo_hbm, xb_hbm, lre_hbm, lim_hbm, bre_hbm, bim_hbm,
            cre_hbm, cim_hbm, ldt_hbm, dsk_hbm, o_hbm,
            xa_s, wq_s, wk_s, wv_s, wt_s, wo_s, lhs_s, w_s, kv_s, kvm_s, oa_s,
            xb_s, v0_s, v1_s, v2_s, v3_s, b_s, c_s, tab_s, inj_s, carry_s, ua_s, ub_s, ob_s,
            phq_s, phi_s, vext_s, ot_s, o_s, sem, osem):
  mk = pltpu.make_async_copy
  vec_l = [v0_s, v1_s, v2_s, v3_s]
  c_vec = [mk(h, s, sem.at[i])
           for i, (h, s) in enumerate(zip((lre_hbm, lim_hbm, ldt_hbm, dsk_hbm), vec_l))]
  c_wt = mk(wt_hbm, wt_s, sem.at[4])
  c_wq = mk(wqkv_hbm.at[:, 0:640], wq_s, sem.at[5])
  c_wk = mk(wqkv_hbm.at[:, 640:1280], wk_s, sem.at[6])
  c_wv = mk(wqkv_hbm.at[:, 1280:1920], wv_s, sem.at[7])
  c_cre = mk(cre_hbm, c_s.at[0], sem.at[8])
  c_cim = mk(cim_hbm, c_s.at[1], sem.at[9])
  c_wo = mk(wo_hbm, wo_s, sem.at[10])
  c_b = [[mk(bre_hbm.at[128 * g0: 128 * g1], b_s.at[128 * g0: 128 * g1], sem.at[11 + 2 * n]),
          mk(bim_hbm.at[128 * g0: 128 * g1], b_s.at[640 + 128 * g0: 640 + 128 * g1],
             sem.at[12 + 2 * n])]
         for n, (g0, g1) in enumerate(BG)]

  def c_xa(i):
    r0 = _mo(i * CA, CA)
    return mk(xa_hbm.at[0, pl.ds(r0, CA)], xa_s.at[pl.ds(r0, CA)], sem.at[17 + i])

  def c_xb(i):
    r0 = _mo(i * CB, CB)
    return mk(xb_hbm.at[0, pl.ds(r0, CB)], xb_s.at[pl.ds(r0, CB)], sem.at[17 + NIT + i])

  def out_b(i):
    r0 = _mo(i * CB, CB)
    return mk(ob_s.at[pl.ds(r0, CB)], o_hbm.at[0, pl.ds(r0, CB), 640:1280], osem.at[0])

  def out_a(i, n):
    r0 = _mo(i * CA, CA)
    cs = slice(128 * n, 128 * n + 128)
    return mk(oa_s.at[pl.ds(r0, CA), cs], o_hbm.at[0, pl.ds(r0, CA), cs], osem.at[1])

  order = c_vec + [c_wt, c_xb(0), c_xb(1)] + c_b[0] + c_b[1] + c_b[2]
  order += [c_xb(2), c_xb(3), c_wk, c_wv, c_wq, c_cre, c_cim, c_xb(NIT), c_xa(0)]
  for i in range(1, NIT):
    order += [c_xa(i), c_xb(NIT + i)]
  order += [c_wo]
  for c in order:
    c.start()

  for c in c_vec:
    c.wait()
  c_wt.wait()

  def vec(i):
    return jnp.broadcast_to(vec_l[i][...].astype(f32).reshape(1, P), (8, P))

  lre, lim, ldt, dsk = vec(0), vec(1), vec(2), vec(3)
  dt = jnp.exp(ldt).astype(bf16).astype(f32)
  mag = jnp.exp(dt * lre)
  lr, li = mag * jnp.cos(dt * lim), mag * jnp.sin(dt * lim)
  sc = jnp.maximum(jnp.abs(lre), jnp.abs(lim))
  sre, sim = lre / sc, lim / sc
  den = (sre * sre + sim * sim) * sc
  cr = ((lr - 1.0) * sre + li * sim) / den
  ci = (li * sre - (lr - 1.0) * sim) / den
  j8 = _iota((8, P), 0)
  pw = [(lr, -li)]
  for _ in range(7):
    pw.append(_cmul(*pw[-1], *pw[0]))
  pr, pi = pw[0]
  for k in range(1, 8):
    pr = jnp.where(j8 == k, pw[k][0], pr)
    pi = jnp.where(j8 == k, pw[k][1], pi)
  for lv in range(3):
    inj_s[2 * lv] = jnp.where(j8 < 2 ** lv, pr, 0.0)
    inj_s[2 * lv + 1] = jnp.where(j8 < 2 ** lv, pi, 0.0)
  for n, s in enumerate((1, 2, 4)):
    tab_s[2 * n] = jnp.where(j8 >= s, pw[s - 1][0], 0.0)
    tab_s[2 * n + 1] = jnp.where(j8 >= s, pw[s - 1][1], 0.0)
  tab_s[6] = dsk
  tab_s[7] = cr * 2.0
  tab_s[8] = ci * 2.0
  carry_s[...] = jnp.zeros_like(carry_s)
  kv_s[...] = jnp.zeros_like(kv_s)
  for j in range(5):
    lhs_s[j] = _fold_lhs(wt_s, j)

  def bu(i, second, cs, nch=1):
    n = CB * nch
    r0 = _mo(i * CB, CB)
    rx = _mo((i + (NIT if second else 0)) * CB, CB)
    u_s = ub_s if second else ua_s
    x = xb_s[pl.ds(rx, n), :]
    for c in cs:
      sl = slice(128 * c, 128 * c + 128)
      ur = _dot(x, b_s[128 * c: 128 * c + 128, :], NT)
      ui = _dot(x, b_s[640 + 128 * c: 640 + 128 * c + 128, :], NT)
      cr2 = tab_s[7, 0:1, sl]
      ci2 = tab_s[8, 0:1, sl]
      u_s[pl.ds(r0, n), sl] = ur * cr2 - ui * ci2
      u_s[pl.ds(r0, n), 640 + 128 * c: 640 + 128 * c + 128] = -(ur * ci2) - ui * cr2

  def scan(i, c, second):
    u_s = ub_s if second else ua_s
    r0 = _mo(i * CB, CB)
    sl = slice(128 * c, 128 * c + 128)
    ur = u_s[pl.ds(r0, CB), sl]
    ui = u_s[pl.ds(r0, CB), 640 + 128 * c: 640 + 128 * c + 128]
    lv = (INJ2 if second else INJ1)[c]
    m = {s: (tab_s[2 * n][:, sl], tab_s[2 * n + 1][:, sl]) for n, s in enumerate((1, 2, 4))}
    ir, ii = inj_s[2 * lv][:, sl], inj_s[2 * lv + 1][:, sl]
    hr = carry_s[0][:, sl]
    hi = carry_s[1][:, sl]

    def rnd(vr, vi, s):
      mr, mi = m[s]
      rr = pltpu.roll(vr, s, 0)
      ri = pltpu.roll(vi, s, 0)
      return vr + (mr * rr - mi * ri), vi + (mr * ri + mi * rr)

    outr, outi = [], []
    for g in range(CB // 8):
      vr = ur[8 * g: 8 * g + 8]
      vi = ui[8 * g: 8 * g + 8]
      for s in (1, 2, 4)[:lv]:
        vr, vi = rnd(vr, vi, s)
      if lv == 0:
        pr_, pi_ = pltpu.roll(hr, 1, 0), pltpu.roll(hi, 1, 0)
      else:
        pr_ = jnp.broadcast_to(hr[7:8, :], (8, 128))
        pi_ = jnp.broadcast_to(hi[7:8, :], (8, 128))
      vr, vi = vr + (ir * pr_ - ii * pi_), vi + (ir * pi_ + ii * pr_)
      for s in (1, 2, 4)[lv:]:
        vr, vi = rnd(vr, vi, s)
      hr, hi = vr, vi
      outr.append(hr)
      outi.append(hi)
    carry_s[0, :, sl] = hr
    carry_s[1, :, sl] = hi
    return jnp.concatenate(outr, 0).astype(bf16), jnp.concatenate(outi, 0).astype(bf16)

  def ypart(i, c, second, yacc):
    ib = i + (NIT if second else 0)
    r0 = _mo(ib * CB, CB)
    sl = slice(128 * c, 128 * c + 128)
    hr, hi = scan(i, c, second)
    y = _dot(hr, c_s[0, :, sl], NT) + _dot(hi, c_s[1, :, sl], NT)
    if c == 0:
      yacc = y + xb_s[pl.ds(r0, CB), :].astype(f32) * tab_s[6, 0:1, :]
    else:
      yacc = yacc + y
    if c == 4:
      ob_s[pl.ds(r0, CB), :] = yacc
      out_b(ib).start()
    return yacc

  c_xb(0).wait()
  c_xb(1).wait()
  for n, (g0, g1) in enumerate(BG):
    c_b[n][0].wait()
    c_b[n][1].wait()
    if n == len(BG) - 1:
      c_xb(2).wait()
      c_xb(3).wait()
    bu(0, False, range(g0, g1), 2)
  bu(2, False, range(5), 2)
  c_wk.wait()
  c_wv.wait()
  c_wq.wait()
  _fold(lhs_s, wk_s, w_s, 1)
  w_s[1280:1920, :] = wv_s[...].T
  _fold(lhs_s, wq_s, w_s, 0)
  c_cre.wait()
  c_cim.wait()

  def body1(i, carry):
    c_xa(i).wait()
    c_xb(NIT + i).wait()
    x = xa_s[pl.ds(_mo(i * CA, CA), CA), :]
    st = {"y": None}
    for tok in ORDER1:
      if tok[0] == "Y":
        st["y"] = ypart(i, int(tok[1]), False, st["y"])
      elif tok[0] == "B":
        bu(i, True, [int(ch) for ch in tok[1:]])
      elif tok[0] == "V":
        k = int(tok[1])
        st[tok] = _dot(w_s[1280 + 320 * k: 1600 + 320 * k, :], x, NT)
      elif tok == "PK":
        st["pk"] = _dot(w_s[640:1280, :], x, NT)
      elif tok == "PQ":
        phq_s[i] = _softmax2(_dot(w_s[0:640, :], x, NT))
      else:
        phi_s[...] = _softmax2(st["pk"])
        vv = jnp.concatenate([st["V0"], st["V1"]], 0).reshape(16, 40, CA)
        vext = jnp.concatenate([vv, jnp.ones((16, 8, CA), f32)], axis=1)
        vext_s[...] = vext.reshape(768, CA).astype(bf16)
        for t, (b0, b1) in enumerate(TB):
          kv_s[TOFF[t]: TOFF[t + 1], :] += _dot(
              vext_s[48 * b0: 48 * (b1 + 1), :], phi_s[128 * t: 128 * t + 128, :], NT)
    return carry

  lax.fori_loop(0, NIT, body1, 0)

  for t, (b0, b1) in enumerate(TB):
    kap = _iota((48, 128), 1) + 128 * t
    hcol = 2 * ((kap * 13108) >> 20) + (kap & 1)
    rr = _iota((48, 128), 0)
    hin = jnp.where(rr < 40, jnp.where(rr < 20, 0, 1), jnp.where(rr < 44, 0, 1))
    for bb in range(b1 - b0 + 1):
      o = TOFF[t] + 48 * bb
      kvm_s[o: o + 48, :] = jnp.where(
          hcol == 2 * (b0 + bb) + hin, kv_s[o: o + 48, :], 0.0).astype(bf16)
  c_wo.wait()

  def body2(i, carry):
    r0 = _mo(i * CA, CA)
    yacc = None
    for tok in ORDER2:
      if tok[0] == "Y":
        yacc = ypart(i, int(tok[1]), True, yacc)
      elif tok[0] == "W":
        n = int(tok[1])
        cs = slice(128 * n, 128 * n + 128)
        oa_s[pl.ds(r0, CA), cs] = _dot(o_s[...], wo_s[:, cs], NN)
        out_a(i, n).start()
      else:
        acc = [None] * 16
        for t, (b0, b1) in enumerate(TB):
          r = _dot(kvm_s[TOFF[t]: TOFF[t + 1], :], phq_s[i, 128 * t: 128 * t + 128, :], NN)
          for bb in range(b1 - b0 + 1):
            piece = r[48 * bb: 48 * bb + 48]
            acc[b0 + bb] = piece if acc[b0 + bb] is None else acc[b0 + bb] + piece
        sub = _iota((8, CA), 0)
        for b in range(16):
          rd = 1.0 / (acc[b][40:48] + 1e-6)
          rs = pltpu.roll(rd, 4, 0)
          r_0 = jnp.where(sub < 4, rd, rs)
          r_1 = jnp.where(sub < 4, rs, rd)
          ot_s[40 * b: 40 * b + 40, :] = acc[b][0:40] * jnp.concatenate(
              [r_0, r_0, rd, r_1, r_1], 0)
        o_s[...] = ot_s[...].astype(bf16).T
    return carry

  lax.fori_loop(0, NIT, body2, 0)

  for i in range(2 * NIT):
    out_b(i).wait()
  for i in range(NIT):
    for n in range(5):
      out_a(i, n).wait()


@jax.jit
def pallas_concat_heads__linear_kernel_hedgehog__ssm_conv_s5__prompt_kernel(
    A_x: jax.Array,
    A_wqkv: jax.Array,
    A_w_phi: jax.Array,
    A_wo: jax.Array,
    B_x: jax.Array,
    B_Lambda_re: jax.Array,
    B_Lambda_im: jax.Array,
    B_B_re: jax.Array,
    B_B_im: jax.Array,
    B_C_re: jax.Array,
    B_C_im: jax.Array,
    B_log_dt: jax.Array,
    B_Dskip: jax.Array,
):
  wt = jnp.transpose(A_w_phi, (1, 2, 0))
  vmem = pltpu.VMEM
  return pl.pallas_call(
      _kernel,
      out_shape=jax.ShapeDtypeStruct((1, S, 2 * D), f32),
      in_specs=[pl.BlockSpec(memory_space=pl.ANY)] * 13,
      out_specs=pl.BlockSpec(memory_space=pl.ANY),
      scratch_shapes=[
          vmem((S, D), bf16), vmem((D, D), bf16), vmem((D, D), bf16), vmem((D, D), bf16),
          vmem((20, 20, 32), bf16), vmem((D, D), bf16), vmem((5, 160, 128), bf16),
          vmem((3 * D, D), bf16), vmem((TOFF[-1], 128), f32), vmem((TOFF[-1], 128), bf16),
          vmem((S, D), f32),
          vmem((S, D), bf16), vmem((P,), bf16), vmem((P,), bf16), vmem((P,), bf16),
          vmem((P,), bf16), vmem((2 * P, D), bf16), vmem((2, D, P), bf16),
          vmem((9, 8, P), f32), vmem((6, 8, P), f32), vmem((2, 8, P), f32),
          vmem((S // 2, 2 * P), f32), vmem((S // 2, 2 * P), f32), vmem((S, D), f32),
          vmem((NIT, 1280, CA), bf16), vmem((1280, CA), bf16), vmem((768, CA), bf16),
          vmem((D, CA), f32), vmem((CA, D), bf16),
          pltpu.SemaphoreType.DMA((17 + 3 * NIT,)), pltpu.SemaphoreType.DMA((2,)),
      ],
      compiler_params=pltpu.CompilerParams(vmem_limit_bytes=100 * 2**20),
  )(A_x, A_wqkv, wt, A_wo, B_x, B_Lambda_re, B_Lambda_im, B_B_re, B_B_im, B_C_re, B_C_im,
    B_log_dt, B_Dskip)
```

```python
import numpy as np

import jax
import jax.numpy as jnp
from jax import lax
import jax.experimental.pallas as pl
import jax.experimental.pallas.tpu as pltpu

S, D, P = 2048, 640, 640
f32, bf16 = jnp.float32, jnp.bfloat16
NT = (((1,), (1,)), ((), ()))
NN = (((1,), (0,)), ((), ()))
LOG2E = 1.4426950408889634
TB = [((128 * t) // 80, (128 * t + 127) // 80) for t in range(10)]
TOFF = np.cumsum([0] + [48 * (b1 - b0 + 1) for b0, b1 in TB]).tolist()

CA = 512
CB = CA // 2
NIT = S // CA
BG = ((0, 1), (1, 3), (3, 5))
ORDER1 = "B01234,Y01,PK,V0,V1,Y234,PQ,KV".split(",")
ORDER2 = "NUM,Y012,W0,W1,Y34,W2,W3,W4".split(",")
INJ1 = (1, 2, 2, 2, 2)
INJ2 = (2, 2, 2, 2, 2)


def _dot(a, b, dn):
  return lax.dot_general(a, b, dn, preferred_element_type=f32)


def _mo(x, n):
  return x if isinstance(x, int) else pl.multiple_of(x, n)


def _cmul(ar, ai, br, bi):
  return ar * br - ai * bi, ar * bi + ai * br


def _iota(shape, dim):
  return lax.broadcasted_iota(jnp.int32, shape, dim)


def _softmax2(p):
  c = p.shape[1]
  x = p.reshape(16, 5, 8, c)

  def allred(m, op):
    m = op(m, pltpu.roll(m, 4, 1))
    return op(m, pltpu.roll(m, 2, 1))[:, None]

  mx = allred(jnp.max(x, axis=1), jnp.maximum)
  mn = allred(jnp.min(x, axis=1), jnp.minimum)
  ep = jnp.exp2(x - mx)
  en = jnp.exp2(mn - x)
  rp = 1.0 / allred(jnp.sum(ep, axis=1), jnp.add)
  rn = 1.0 / allred(jnp.sum(en, axis=1), jnp.add)
  phi = jnp.concatenate([ep * rp, en * rn], axis=1)
  return phi.reshape(1280, c).astype(bf16)


def _fold_lhs(wt_s, j):
  r = _iota((32, 128), 1) + 128 * j
  hr = (r * 3277) >> 16
  e = jnp.where(_iota((32, 128), 0) == hr, 1.0, 0.0).astype(bf16)
  dr1 = (r - 20 * hr)[0:1, :]
  t = jnp.zeros((20, 128), f32)
  for d in range(20):
    t = jnp.where(dr1 == d, _dot(wt_s[d], e, NN), t)
  dup = jnp.where(_iota((40, 20), 0) >> 1 == _iota((40, 20), 1), 1.0, 0.0).astype(bf16)
  t2 = _dot(dup, t.astype(bf16), NN)
  h2 = _iota((40, 128), 0) & 1
  hr1 = hr[0:1, :]
  return jnp.concatenate(
      [jnp.where(2 * (3 * j + bb) + h2 == hr1, t2, 0.0) for bb in range(4)], 0).astype(bf16)


def _fold(lhs_s, w_ref, wt_out, n):
  prev = None
  for j in range(5):
    res = _dot(lhs_s[j], w_ref[:, 128 * j: 128 * j + 128], NT) * LOG2E
    lo = 640 * n + 120 * j
    if j == 0:
      wt_out[lo: lo + 120, :] = res[0:120].astype(bf16)
    else:
      wt_out[lo: lo + 40, :] = (prev + res[0:40]).astype(bf16)
      wt_out[lo + 40: lo + 120, :] = res[40:120].astype(bf16)
    if j < 4:
      prev = res[120:160]
    else:
      wt_out[lo + 120: lo + 160, :] = res[120:160].astype(bf16)


def _kernel(xa_hbm, wqkv_hbm, wt_hbm, wo_hbm, xb_hbm, lre_hbm, lim_hbm, bre_hbm, bim_hbm,
            cre_hbm, cim_hbm, ldt_hbm, dsk_hbm, o_hbm,
            xa_s, wq_s, wk_s, wv_s, wt_s, wo_s, lhs_s, w_s, kv_s, kvm_s, oa_s,
            xb_s, v0_s, v1_s, v2_s, v3_s, b_s, c_s, tab_s, inj_s, carry_s, ua_s, ub_s, ob_s,
            phq_s, phi_s, vext_s, ot_s, o_s, sem, osem):
  mk = pltpu.make_async_copy
  vec_l = [v0_s, v1_s, v2_s, v3_s]
  c_vec = [mk(h, s, sem.at[i])
           for i, (h, s) in enumerate(zip((lre_hbm, lim_hbm, ldt_hbm, dsk_hbm), vec_l))]
  c_wt = mk(wt_hbm, wt_s, sem.at[4])
  c_wq = mk(wqkv_hbm.at[:, 0:640], wq_s, sem.at[5])
  c_wk = mk(wqkv_hbm.at[:, 640:1280], wk_s, sem.at[6])
  c_wv = mk(wqkv_hbm.at[:, 1280:1920], wv_s, sem.at[7])
  c_cre = mk(cre_hbm, c_s.at[0], sem.at[8])
  c_cim = mk(cim_hbm, c_s.at[1], sem.at[9])
  c_wo = mk(wo_hbm, wo_s, sem.at[10])
  c_b = [[mk(bre_hbm.at[128 * g0: 128 * g1], b_s.at[128 * g0: 128 * g1], sem.at[11 + 2 * n]),
          mk(bim_hbm.at[128 * g0: 128 * g1], b_s.at[640 + 128 * g0: 640 + 128 * g1],
             sem.at[12 + 2 * n])]
         for n, (g0, g1) in enumerate(BG)]

  def c_xa(i):
    r0 = _mo(i * CA, CA)
    return mk(xa_hbm.at[0, pl.ds(r0, CA)], xa_s.at[pl.ds(r0, CA)], sem.at[17 + i])

  def c_xb(i):
    r0 = _mo(i * CB, CB)
    return mk(xb_hbm.at[0, pl.ds(r0, CB)], xb_s.at[pl.ds(r0, CB)], sem.at[17 + NIT + i])

  def out_b(i):
    r0 = _mo(i * CB, CB)
    return mk(ob_s.at[pl.ds(r0, CB)], o_hbm.at[0, pl.ds(r0, CB), 640:1280], osem.at[0])

  def out_a(i, n):
    r0 = _mo(i * CA, CA)
    cs = slice(128 * n, 128 * n + 128)
    return mk(oa_s.at[pl.ds(r0, CA), cs], o_hbm.at[0, pl.ds(r0, CA), cs], osem.at[1])

  order = c_vec + [c_wt, c_xb(0), c_xb(1)] + c_b[0] + c_b[1] + c_b[2]
  order += [c_xb(2), c_xb(3), c_wk, c_wv, c_wq, c_cre, c_cim, c_xb(NIT), c_xa(0)]
  for i in range(1, NIT):
    order += [c_xa(i), c_xb(NIT + i)]
  order += [c_wo]
  for c in order:
    c.start()

  for c in c_vec:
    c.wait()
  c_wt.wait()

  def vec(i):
    return jnp.broadcast_to(vec_l[i][...].astype(f32).reshape(1, P), (8, P))

  lre, lim, ldt, dsk = vec(0), vec(1), vec(2), vec(3)
  dt = jnp.exp(ldt).astype(bf16).astype(f32)
  mag = jnp.exp(dt * lre)
  lr, li = mag * jnp.cos(dt * lim), mag * jnp.sin(dt * lim)
  sc = jnp.maximum(jnp.abs(lre), jnp.abs(lim))
  sre, sim = lre / sc, lim / sc
  den = (sre * sre + sim * sim) * sc
  cr = ((lr - 1.0) * sre + li * sim) / den
  ci = (li * sre - (lr - 1.0) * sim) / den
  j8 = _iota((8, P), 0)
  pw = [(lr, -li)]
  for _ in range(7):
    pw.append(_cmul(*pw[-1], *pw[0]))
  pr, pi = pw[0]
  for k in range(1, 8):
    pr = jnp.where(j8 == k, pw[k][0], pr)
    pi = jnp.where(j8 == k, pw[k][1], pi)
  for lv in range(3):
    inj_s[2 * lv] = jnp.where(j8 < 2 ** lv, pr, 0.0)
    inj_s[2 * lv + 1] = jnp.where(j8 < 2 ** lv, pi, 0.0)
  for n, s in enumerate((1, 2, 4)):
    tab_s[2 * n] = jnp.where(j8 >= s, pw[s - 1][0], 0.0)
    tab_s[2 * n + 1] = jnp.where(j8 >= s, pw[s - 1][1], 0.0)
  tab_s[6] = dsk
  tab_s[7] = cr * 2.0
  tab_s[8] = ci * 2.0
  carry_s[...] = jnp.zeros_like(carry_s)
  kv_s[...] = jnp.zeros_like(kv_s)
  for j in range(5):
    lhs_s[j] = _fold_lhs(wt_s, j)

  def bu(i, second, cs, nch=1):
    n = CB * nch
    r0 = _mo(i * CB, CB)
    rx = _mo((i + (NIT if second else 0)) * CB, CB)
    u_s = ub_s if second else ua_s
    x = xb_s[pl.ds(rx, n), :]
    for c in cs:
      sl = slice(128 * c, 128 * c + 128)
      ur = _dot(x, b_s[128 * c: 128 * c + 128, :], NT)
      ui = _dot(x, b_s[640 + 128 * c: 640 + 128 * c + 128, :], NT)
      cr2 = tab_s[7, 0:1, sl]
      ci2 = tab_s[8, 0:1, sl]
      u_s[pl.ds(r0, n), sl] = ur * cr2 - ui * ci2
      u_s[pl.ds(r0, n), 640 + 128 * c: 640 + 128 * c + 128] = -(ur * ci2) - ui * cr2

  def scan(i, c, second):
    u_s = ub_s if second else ua_s
    r0 = _mo(i * CB, CB)
    sl = slice(128 * c, 128 * c + 128)
    ur = u_s[pl.ds(r0, CB), sl]
    ui = u_s[pl.ds(r0, CB), 640 + 128 * c: 640 + 128 * c + 128]
    lv = (INJ2 if second else INJ1)[c]
    m = {s: (tab_s[2 * n][:, sl], tab_s[2 * n + 1][:, sl]) for n, s in enumerate((1, 2, 4))}
    ir, ii = inj_s[2 * lv][:, sl], inj_s[2 * lv + 1][:, sl]
    hr = carry_s[0][:, sl]
    hi = carry_s[1][:, sl]

    def rnd(vr, vi, s):
      mr, mi = m[s]
      rr = pltpu.roll(vr, s, 0)
      ri = pltpu.roll(vi, s, 0)
      return vr + (mr * rr - mi * ri), vi + (mr * ri + mi * rr)

    outr, outi = [], []
    for g in range(CB // 8):
      vr = ur[8 * g: 8 * g + 8]
      vi = ui[8 * g: 8 * g + 8]
      for s in (1, 2, 4)[:lv]:
        vr, vi = rnd(vr, vi, s)
      if lv == 0:
        pr_, pi_ = pltpu.roll(hr, 1, 0), pltpu.roll(hi, 1, 0)
      else:
        pr_ = jnp.broadcast_to(hr[7:8, :], (8, 128))
        pi_ = jnp.broadcast_to(hi[7:8, :], (8, 128))
      vr, vi = vr + (ir * pr_ - ii * pi_), vi + (ir * pi_ + ii * pr_)
      for s in (1, 2, 4)[lv:]:
        vr, vi = rnd(vr, vi, s)
      hr, hi = vr, vi
      outr.append(hr)
      outi.append(hi)
    carry_s[0, :, sl] = hr
    carry_s[1, :, sl] = hi
    return jnp.concatenate(outr, 0).astype(bf16), jnp.concatenate(outi, 0).astype(bf16)

  def ypart(i, cs, second, yacc):
    ib = i + (NIT if second else 0)
    r0 = _mo(ib * CB, CB)
    hs = [scan(i, c, second) for c in cs]
    y = None
    for c, (hr, hi) in zip(cs, hs):
      sl = slice(128 * c, 128 * c + 128)
      yc = _dot(hr, c_s[0, :, sl], NT) + _dot(hi, c_s[1, :, sl], NT)
      y = yc if y is None else y + yc
    if 0 in cs:
      yacc = y + xb_s[pl.ds(r0, CB), :].astype(f32) * tab_s[6, 0:1, :]
    else:
      yacc = yacc + y
    if 4 in cs:
      ob_s[pl.ds(r0, CB), :] = yacc
      out_b(ib).start()
    return yacc

  c_xb(0).wait()
  c_xb(1).wait()
  for n, (g0, g1) in enumerate(BG):
    c_b[n][0].wait()
    c_b[n][1].wait()
    if n == len(BG) - 1:
      c_xb(2).wait()
      c_xb(3).wait()
    bu(0, False, range(g0, g1), 2)
  bu(2, False, range(5), 2)
  c_wk.wait()
  c_wv.wait()
  c_wq.wait()
  _fold(lhs_s, wk_s, w_s, 1)
  w_s[1280:1920, :] = wv_s[...].T
  _fold(lhs_s, wq_s, w_s, 0)
  c_cre.wait()
  c_cim.wait()

  def body1(i, carry):
    c_xa(i).wait()
    c_xb(NIT + i).wait()
    x = xa_s[pl.ds(_mo(i * CA, CA), CA), :]
    st = {"y": None}
    for tok in ORDER1:
      if tok[0] == "Y":
        st["y"] = ypart(i, [int(ch) for ch in tok[1:]], False, st["y"])
      elif tok[0] == "B":
        bu(i, True, [int(ch) for ch in tok[1:]])
      elif tok[0] == "V":
        k = int(tok[1])
        st[tok] = _dot(w_s[1280 + 320 * k: 1600 + 320 * k, :], x, NT)
      elif tok == "PK":
        st["pk"] = _dot(w_s[640:1280, :], x, NT)
      elif tok == "PQ":
        phq_s[i] = _softmax2(_dot(w_s[0:640, :], x, NT))
      else:
        phi_s[...] = _softmax2(st["pk"])
        vv = jnp.concatenate([st["V0"], st["V1"]], 0).reshape(16, 40, CA)
        vext = jnp.concatenate([vv, jnp.ones((16, 8, CA), f32)], axis=1)
        vext_s[...] = vext.reshape(768, CA).astype(bf16)
        for t, (b0, b1) in enumerate(TB):
          kv_s[TOFF[t]: TOFF[t + 1], :] += _dot(
              vext_s[48 * b0: 48 * (b1 + 1), :], phi_s[128 * t: 128 * t + 128, :], NT)
    return carry

  lax.fori_loop(0, NIT, body1, 0)

  for t, (b0, b1) in enumerate(TB):
    kap = _iota((48, 128), 1) + 128 * t
    hcol = 2 * ((kap * 13108) >> 20) + (kap & 1)
    rr = _iota((48, 128), 0)
    hin = jnp.where(rr < 40, jnp.where(rr < 20, 0, 1), jnp.where(rr < 44, 0, 1))
    for bb in range(b1 - b0 + 1):
      o = TOFF[t] + 48 * bb
      kvm_s[o: o + 48, :] = jnp.where(
          hcol == 2 * (b0 + bb) + hin, kv_s[o: o + 48, :], 0.0).astype(bf16)
  c_wo.wait()

  def body2(i, carry):
    r0 = _mo(i * CA, CA)
    yacc = None
    for tok in ORDER2:
      if tok[0] == "Y":
        yacc = ypart(i, [int(ch) for ch in tok[1:]], True, yacc)
      elif tok[0] == "W":
        n = int(tok[1])
        cs = slice(128 * n, 128 * n + 128)
        oa_s[pl.ds(r0, CA), cs] = _dot(o_s[...], wo_s[:, cs], NN)
        out_a(i, n).start()
      else:
        acc = [None] * 16
        for t, (b0, b1) in enumerate(TB):
          r = _dot(kvm_s[TOFF[t]: TOFF[t + 1], :], phq_s[i, 128 * t: 128 * t + 128, :], NN)
          for bb in range(b1 - b0 + 1):
            piece = r[48 * bb: 48 * bb + 48]
            acc[b0 + bb] = piece if acc[b0 + bb] is None else acc[b0 + bb] + piece
        sub = _iota((8, CA), 0)
        for b in range(16):
          rd = 1.0 / (acc[b][40:48] + 1e-6)
          rs = pltpu.roll(rd, 4, 0)
          r_0 = jnp.where(sub < 4, rd, rs)
          r_1 = jnp.where(sub < 4, rs, rd)
          ot_s[40 * b: 40 * b + 40, :] = acc[b][0:40] * jnp.concatenate(
              [r_0, r_0, rd, r_1, r_1], 0)
        o_s[...] = ot_s[...].astype(bf16).T
    return carry

  lax.fori_loop(0, NIT, body2, 0)

  for i in range(2 * NIT):
    out_b(i).wait()
  for i in range(NIT):
    for n in range(5):
      out_a(i, n).wait()


@jax.jit
def pallas_concat_heads__linear_kernel_hedgehog__ssm_conv_s5__prompt_kernel(
    A_x: jax.Array,
    A_wqkv: jax.Array,
    A_w_phi: jax.Array,
    A_wo: jax.Array,
    B_x: jax.Array,
    B_Lambda_re: jax.Array,
    B_Lambda_im: jax.Array,
    B_B_re: jax.Array,
    B_B_im: jax.Array,
    B_C_re: jax.Array,
    B_C_im: jax.Array,
    B_log_dt: jax.Array,
    B_Dskip: jax.Array,
):
  wt = jnp.transpose(A_w_phi, (1, 2, 0))
  vmem = pltpu.VMEM
  return pl.pallas_call(
      _kernel,
      out_shape=jax.ShapeDtypeStruct((1, S, 2 * D), f32),
      in_specs=[pl.BlockSpec(memory_space=pl.ANY)] * 13,
      out_specs=pl.BlockSpec(memory_space=pl.ANY),
      scratch_shapes=[
          vmem((S, D), bf16), vmem((D, D), bf16), vmem((D, D), bf16), vmem((D, D), bf16),
          vmem((20, 20, 32), bf16), vmem((D, D), bf16), vmem((5, 160, 128), bf16),
          vmem((3 * D, D), bf16), vmem((TOFF[-1], 128), f32), vmem((TOFF[-1], 128), bf16),
          vmem((S, D), f32),
          vmem((S, D), bf16), vmem((P,), bf16), vmem((P,), bf16), vmem((P,), bf16),
          vmem((P,), bf16), vmem((2 * P, D), bf16), vmem((2, D, P), bf16),
          vmem((9, 8, P), f32), vmem((6, 8, P), f32), vmem((2, 8, P), f32),
          vmem((S // 2, 2 * P), f32), vmem((S // 2, 2 * P), f32), vmem((S, D), f32),
          vmem((NIT, 1280, CA), bf16), vmem((1280, CA), bf16), vmem((768, CA), bf16),
          vmem((D, CA), f32), vmem((CA, D), bf16),
          pltpu.SemaphoreType.DMA((17 + 3 * NIT,)), pltpu.SemaphoreType.DMA((2,)),
      ],
      compiler_params=pltpu.CompilerParams(vmem_limit_bytes=100 * 2**20),
  )(A_x, A_wqkv, wt, A_wo, B_x, B_Lambda_re, B_Lambda_im, B_B_re, B_B_im, B_C_re, B_C_im,
    B_log_dt, B_Dskip)
```
